```python
import os as _os
_os.environ.setdefault("JAX_PLATFORMS", "cpu")
import jax
import jax.numpy as jnp

def _softmax(x, axis=-1):
    return jax.nn.softmax(x, axis=axis)
def _gelu(x):
    return jax.nn.gelu(x, approximate=True)
def _silu(x):
    return jax.nn.silu(x)
def _sigmoid(x):
    return jax.nn.sigmoid(x)
def _layernorm(x, axis=-1, eps=1e-5):
    m = jnp.mean(x, axis=axis, keepdims=True)
    v = jnp.var(x, axis=axis, keepdims=True)
    return (x - m) / jnp.sqrt(v + eps)
def _scatter_add(tgt, idx, src, axis=0):
    return tgt.at[idx].add(src)
def _segment_sum(src, seg, n):
    return jax.ops.segment_sum(src, seg, n)
class _Rng:
    def __init__(self, key):
        self._k = key
    def _next(self):
        self._k, sub = jax.random.split(self._k)
        return sub
    def normal(self, shape):
        return jax.random.normal(self._next(), shape, dtype=jnp.bfloat16)
    def randint(self, lo, hi, shape):
        return jax.random.randint(self._next(), shape, lo, hi, dtype=jnp.int32)
    def uniform(self, shape, lo=0.0, hi=1.0):
        return jax.random.uniform(self._next(), shape, jnp.bfloat16, lo, hi)
    def permutation(self, n):
        return jax.random.permutation(self._next(), n)


kernel_name = 'parallel_sum__mha_block__swiglu_ffn__prompt'

def setup_inputs():
    _rng = _Rng(jax.random.key(int.from_bytes(__import__("os").urandom(4), "little")))
    _w = (lambda a: (lambda t: t.astype(jnp.bfloat16) if jnp.issubdtype(t.dtype, jnp.floating) else t)(jnp.asarray(a)))
    def _A_setup():
        B, S, D, H = 1, 2048, 512, 32
        return {
            "x": _w((lambda *s: _rng.normal(s) * 0.05)(B, S, D)),
            "wqkv": _w((lambda *s: _rng.normal(s) * 0.1)(D, 3 * D)),
            "wo": _w((lambda *s: _rng.normal(s) * 0.05)(D, D)),
        }
    _A_in = _A_setup()

    def _B_setup():
        B, S, D, F = 1, 2048, 512, 1792
        return {
            "x": _w((lambda *s: _rng.normal(s) * 0.05)(B, S, D)),
            "w_gate": _w((lambda *s: _rng.normal(s) * 0.05)(D, F)),
            "w_up": _w((lambda *s: _rng.normal(s) * 0.05)(D, F)),
            "w_down": _w((lambda *s: _rng.normal(s) * 0.05)(F, D)),
        }
    _B_in = _B_setup()

    return {
        "A_x": _A_in["x"],
        "A_wqkv": _A_in["wqkv"],
        "A_wo": _A_in["wo"],
        "B_x": _B_in["x"],
        "B_w_gate": _B_in["w_gate"],
        "B_w_up": _B_in["w_up"],
        "B_w_down": _B_in["w_down"],
    }

def reference(A_x, A_wqkv, A_wo, B_x, B_w_gate, B_w_up, B_w_down):
    def _A_ref(x, wqkv, wo):
        B, S, D = x.shape
        H = 32
        Dh = D // H
        qkv = (lambda x, *d: x.transpose(*d))((x @ wqkv).reshape(B, S, 3, H, Dh), 2, 0, 3, 1, 4)
        q, k, v = qkv[0], qkv[1], qkv[2]
        scores = jnp.einsum("bhqd,bhkd->bhqk", q, k) * (Dh ** -0.5)
        p = _softmax(scores, axis=-1)
        o = jnp.einsum("bhqk,bhkd->bhqd", p, v)
        return (lambda x, *d: x.transpose(*d))(o, 0, 2, 1, 3).reshape(B, S, D) @ wo

    def _B_ref(x, w_gate, w_up, w_down):
        g = _silu(x @ w_gate)
        u = x @ w_up
        return (g * u) @ w_down

    x = A_x
    xn = _layernorm(x, axis=-1)
    return x + _A_ref(xn, A_wqkv, A_wo) + _B_ref(xn, B_w_gate, B_w_up, B_w_down)
```

```python
import functools
import math

import jax
import jax.numpy as jnp
import jax.experimental.pallas as pl
import jax.experimental.pallas.tpu as pltpu

_H = 32
_DH = 16
_LOG2E = math.log2(math.e)
_RC = 512
_L_LO = 2.0 ** -10
_L_HI = 2.0 ** 100


def _f32dot(a, b):
    return jnp.dot(a, b, preferred_element_type=jnp.float32)


def _kernel(x_hbm, wqkv_hbm, wo_hbm, wg_hbm, wu_hbm, wd_hbm, o_ref,
            x_s, wqkv_s, wo_s, wg_s, wu_s, wd_s,
            xn_s, k_s, vt_s, qt_s, ot_s, sems, *, TQ, CK, UNROLL, MODE):
    S, D = x_s.shape
    i = pl.program_id(0)
    NC = S // _RC

    def x_copy(r):
        return pltpu.make_async_copy(x_hbm.at[pl.ds(r * _RC, _RC), :],
                                     x_s.at[pl.ds(r * _RC, _RC), :], sems.at[r])
    w_copies = [pltpu.make_async_copy(src, dst, sems.at[NC + j]) for j, (src, dst) in enumerate(
        [(wqkv_hbm, wqkv_s), (wo_hbm, wo_s), (wg_hbm, wg_s), (wu_hbm, wu_s), (wd_hbm, wd_s)])]

    @pl.when(i == 0)
    def _():
        x_copy(0).start()
        w_copies[0].start()
        for r in range(1, NC):
            x_copy(r).start()
        for c in w_copies[1:]:
            c.start()
        w_copies[0].wait()
        for r in range(NC):
            x_copy(r).wait()
            r0 = r * _RC
            x = x_s[r0:r0 + _RC, :].astype(jnp.float32)
            m = jnp.mean(x, axis=-1, keepdims=True)
            xc = x - m
            v = jnp.mean(xc * xc, axis=-1, keepdims=True)
            xn = (xc * jax.lax.rsqrt(v + 1e-5)).astype(jnp.bfloat16)
            xn_s[r0:r0 + _RC, :] = xn
            kk = _f32dot(xn, wqkv_s[:, D:2 * D]).astype(jnp.bfloat16)
            for b in range(D // 128):
                k_s[b, r0:r0 + _RC, :] = kk[:, b * 128:(b + 1) * 128]
            vv = _f32dot(xn, wqkv_s[:, 2 * D:3 * D])
            vt_s[:, r0:r0 + _RC] = vv.T.astype(jnp.bfloat16)

    q0 = pl.multiple_of(i * TQ, TQ)
    xn_t = xn_s[pl.ds(q0, TQ), :]
    q = _f32dot(xn_t, wqkv_s[:, 0:D]) * (_DH ** -0.5 * _LOG2E)
    qt_s[...] = q.T.astype(jnp.bfloat16)

    row_head = jax.lax.broadcasted_iota(jnp.int32, (128, TQ), 0) // _DH

    def scores(h):
        b = h // 8
        qb = qt_s[pl.ds(pl.multiple_of(b * 128, 128), 128), :]
        rhs = jnp.where(row_head == (h % 8), qb, jnp.zeros_like(qb))
        return [_f32dot(k_s[b, c0:c0 + CK, :], rhs) for c0 in range(0, S, CK)]

    def softmax_pv(h, ss, m):
        v0 = pl.multiple_of(h * _DH, _DH)
        acc = l = None
        for j, s in enumerate(ss):
            p = jnp.exp2(s if m is None else s - m)
            lj = jnp.sum(p, axis=0, keepdims=True)
            oj = _f32dot(vt_s[pl.ds(v0, _DH), j * CK:(j + 1) * CK], p.astype(jnp.bfloat16))
            acc = oj if acc is None else acc + oj
            l = lj if l is None else l + lj
        ot_s[pl.ds(v0, _DH), :] = acc / l
        return acc, l

    def head_fast(h, bad):
        acc, l = softmax_pv(h, scores(h), None)
        ok = (l >= _L_LO) & (l <= _L_HI) & (jnp.max(jnp.abs(acc), axis=0, keepdims=True) <= _L_HI)
        return jnp.where(ok, bad, 1.0)

    def head_safe(h, c):
        ss = scores(h)
        m = functools.reduce(jnp.maximum, [jnp.max(s, axis=0, keepdims=True) for s in ss])
        softmax_pv(h, ss, m)
        return c

    if 'noattn' in MODE:
        ot_s[...] = qt_s[...].astype(jnp.float32)
    elif 'safe' in MODE:
        jax.lax.fori_loop(0, _H, head_safe, 0, unroll=UNROLL)
    else:
        bad = jax.lax.fori_loop(0, _H, head_fast, jnp.zeros((1, TQ), jnp.float32), unroll=UNROLL)

        @pl.when(jnp.max(bad) > 0.0)
        def _():
            jax.lax.fori_loop(0, _H, head_safe, 0)

    @pl.when(i == 0)
    def _():
        for c in w_copies[1:]:
            c.wait()

    o = ot_s[...].T.astype(jnp.bfloat16)
    attn = _f32dot(o, wo_s[...])
    g = _f32dot(xn_t, wg_s[...])
    u = _f32dot(xn_t, wu_s[...])
    hmid = (g * jax.nn.sigmoid(g) * u).astype(jnp.bfloat16)
    f = _f32dot(hmid, wd_s[...])
    o_ref[...] = (x_s[pl.ds(q0, TQ), :].astype(jnp.float32) + attn + f).astype(o_ref.dtype)


def _call(A_x, A_wqkv, A_wo, B_w_gate, B_w_up, B_w_down, TQ=512, CK=256, UNROLL=2, MODE=''):
    B, S, D = A_x.shape
    F = B_w_gate.shape[1]
    bf = jnp.bfloat16
    out = pl.pallas_call(
        functools.partial(_kernel, TQ=TQ, CK=CK, UNROLL=UNROLL, MODE=MODE),
        grid=(S // TQ,),
        in_specs=[pl.BlockSpec(memory_space=pl.ANY)] * 6,
        out_specs=pl.BlockSpec((TQ, D), lambda i: (i, 0)),
        out_shape=jax.ShapeDtypeStruct((S, D), A_x.dtype),
        scratch_shapes=[
            pltpu.VMEM((S, D), A_x.dtype),
            pltpu.VMEM((D, 3 * D), A_wqkv.dtype),
            pltpu.VMEM((D, D), A_wo.dtype),
            pltpu.VMEM((D, F), B_w_gate.dtype),
            pltpu.VMEM((D, F), B_w_up.dtype),
            pltpu.VMEM((F, D), B_w_down.dtype),
            pltpu.VMEM((S, D), bf),
            pltpu.VMEM((D // 128, S, 128), bf),
            pltpu.VMEM((D, S), bf),
            pltpu.VMEM((D, TQ), bf),
            pltpu.VMEM((D, TQ), jnp.float32),
            pltpu.SemaphoreType.DMA((S // _RC + 5,)),
        ],
        compiler_params=pltpu.CompilerParams(
            dimension_semantics=("arbitrary",),
            vmem_limit_bytes=100 * 1024 * 1024),
    )(A_x.reshape(S, D), A_wqkv, A_wo, B_w_gate, B_w_up, B_w_down)
    return out.reshape(B, S, D)


@jax.jit
def pallas_parallel_sum__mha_block__swiglu_ffn__prompt_kernel(
    A_x, A_wqkv, A_wo, B_x, B_w_gate, B_w_up, B_w_down,
):
    return _call(A_x, A_wqkv, A_wo, B_w_gate, B_w_up, B_w_down)
```

```python
import functools
import math

import jax
import jax.numpy as jnp
import jax.experimental.pallas as pl
import jax.experimental.pallas.tpu as pltpu

_H = 32
_DH = 16
_LOG2E = math.log2(math.e)
_RC = 512
_L_LO = 2.0 ** -10
_L_HI = 2.0 ** 100


def _f32dot(a, b):
    return jnp.dot(a, b, preferred_element_type=jnp.float32)


def _kernel(x_hbm, wqkv_hbm, wo_hbm, wg_hbm, wu_hbm, wd_hbm, o_ref,
            x_s, wqkv_s, wo_s, wg_s, wu_s, wd_s,
            xn_s, k_s, vt_s, qt_s, ot_s, sems, *, TQ, CK, UNROLL, LAG):
    S, D = x_s.shape
    i = pl.program_id(0)
    NC = S // _RC

    def x_copy(r):
        return pltpu.make_async_copy(x_hbm.at[pl.ds(r * _RC, _RC), :],
                                     x_s.at[pl.ds(r * _RC, _RC), :], sems.at[r])
    w_copies = [pltpu.make_async_copy(src, dst, sems.at[NC + j]) for j, (src, dst) in enumerate(
        [(wqkv_hbm.at[:, D:2 * D], wqkv_s.at[:, D:2 * D]), (wqkv_hbm.at[:, 2 * D:], wqkv_s.at[:, 2 * D:]),
         (wqkv_hbm.at[:, :D], wqkv_s.at[:, :D]), (wo_hbm, wo_s), (wg_hbm, wg_s), (wu_hbm, wu_s), (wd_hbm, wd_s)])]

    def v_proj(r0):
        vv = _f32dot(xn_s[r0:r0 + _RC, :], wqkv_s[:, 2 * D:3 * D])
        vt_s[:, r0:r0 + _RC] = vv.T.astype(jnp.bfloat16)

    @pl.when(i == 0)
    def _():
        x_copy(0).start()
        w_copies[0].start()
        w_copies[1].start()
        for r in range(1, NC):
            x_copy(r).start()
        for c in w_copies[2:]:
            c.start()
        w_copies[0].wait()
        w_copies[1].wait()
        for r in range(NC):
            if r == 0:
                x_copy(0).wait()
            elif r == 1:
                for rr in range(1, NC):
                    x_copy(rr).wait()
            r0 = r * _RC
            if r > 0:
                v_proj(r0 - _RC)
            x = x_s[r0:r0 + _RC, :].astype(jnp.float32)
            m = jnp.mean(x, axis=-1, keepdims=True)
            xc = x - m
            v = jnp.mean(xc * xc, axis=-1, keepdims=True)
            xn = (xc * jax.lax.rsqrt(v + 1e-5)).astype(jnp.bfloat16)
            xn_s[r0:r0 + _RC, :] = xn
            kk = _f32dot(xn, wqkv_s[:, D:2 * D]).astype(jnp.bfloat16)
            for b in range(D // 128):
                k_s[b, r0:r0 + _RC, :] = kk[:, b * 128:(b + 1) * 128]
        v_proj(S - _RC)
        w_copies[2].wait()

    q0 = pl.multiple_of(i * TQ, TQ)
    xn_t = xn_s[pl.ds(q0, TQ), :]
    q = _f32dot(xn_t, wqkv_s[:, 0:D]) * (_DH ** -0.5 * _LOG2E)
    qt_s[...] = q.T.astype(jnp.bfloat16)

    row_head = jax.lax.broadcasted_iota(jnp.int32, (128, TQ), 0) // _DH

    def scores(h):
        b = h // 8
        qb = qt_s[pl.ds(pl.multiple_of(b * 128, 128), 128), :]
        rhs = jnp.where(row_head == (h % 8), qb, jnp.zeros_like(qb))
        return [_f32dot(k_s[b, c0:c0 + CK, :], rhs) for c0 in range(0, S, CK)]

    def softmax_pv(h, ss, m):
        v0 = pl.multiple_of(h * _DH, _DH)
        acc = l = None
        for j, s in enumerate(ss):
            p = jnp.exp2(s - m)
            lj = jnp.sum(p, axis=0, keepdims=True)
            oj = _f32dot(vt_s[pl.ds(v0, _DH), j * CK:(j + 1) * CK], p.astype(jnp.bfloat16))
            acc = oj if acc is None else acc + oj
            l = lj if l is None else l + lj
        ot_s[pl.ds(v0, _DH), :] = acc / l
        return acc, l

    def masked_q(h):
        qb = qt_s[pl.ds(pl.multiple_of((h // 8) * 128, 128), 128), :]
        return jnp.where(row_head == (h % 8), qb, jnp.zeros_like(qb))

    def group(g, bad):
        NCH = S // CK
        tasks = [(u, j) for u in range(UNROLL) for j in range(NCH)]
        rhs, pend, st = {}, {}, {}

        def issue(t):
            u, j = tasks[t]
            h = g * UNROLL + u
            if u not in rhs:
                rhs[u] = masked_q(h)
            pend[t] = _f32dot(k_s[h // 8, j * CK:(j + 1) * CK, :], rhs[u])

        for t in range(min(LAG, len(tasks))):
            issue(t)
        for t, (u, j) in enumerate(tasks):
            if t + LAG < len(tasks):
                issue(t + LAG)
            h = g * UNROLL + u
            v0 = pl.multiple_of(h * _DH, _DH)
            p = jnp.exp2(pend.pop(t))
            lj = jnp.sum(p, axis=0, keepdims=True)
            oj = _f32dot(vt_s[pl.ds(v0, _DH), j * CK:(j + 1) * CK], p.astype(jnp.bfloat16))
            acc, l = (oj, lj) if j == 0 else (st[u][0] + oj, st[u][1] + lj)
            st[u] = (acc, l)
            if j == NCH - 1:
                ot_s[pl.ds(v0, _DH), :] = acc / l
                ok = ((l >= _L_LO) & (l <= _L_HI)
                      & (jnp.max(jnp.abs(acc), axis=0, keepdims=True) <= _L_HI))
                bad = jnp.where(ok, bad, 1.0)
        return bad

    def head_safe(h, c):
        ss = scores(h)
        m = functools.reduce(jnp.maximum, [jnp.max(s, axis=0, keepdims=True) for s in ss])
        softmax_pv(h, ss, m)
        return c

    bad = jax.lax.fori_loop(0, _H // UNROLL, group, jnp.zeros((1, TQ), jnp.float32))

    @pl.when(jnp.max(bad) > 0.0)
    def _():
        jax.lax.fori_loop(0, _H, head_safe, 0)

    @pl.when(i == 0)
    def _():
        for c in w_copies[3:]:
            c.wait()

    g = _f32dot(xn_t, wg_s[...])
    u = _f32dot(xn_t, wu_s[...])
    o = ot_s[...].T.astype(jnp.bfloat16)
    hmid = (g * jax.nn.sigmoid(g) * u).astype(jnp.bfloat16)
    attn = _f32dot(o, wo_s[...])
    f = _f32dot(hmid, wd_s[...])
    o_ref[...] = (x_s[pl.ds(q0, TQ), :].astype(jnp.float32) + attn + f).astype(o_ref.dtype)


def _call(A_x, A_wqkv, A_wo, B_w_gate, B_w_up, B_w_down, TQ=512, CK=128, UNROLL=8, LAG=2):
    B, S, D = A_x.shape
    F = B_w_gate.shape[1]
    bf = jnp.bfloat16
    out = pl.pallas_call(
        functools.partial(_kernel, TQ=TQ, CK=CK, UNROLL=UNROLL, LAG=LAG),
        grid=(S // TQ,),
        in_specs=[pl.BlockSpec(memory_space=pl.ANY)] * 6,
        out_specs=pl.BlockSpec((TQ, D), lambda i: (i, 0)),
        out_shape=jax.ShapeDtypeStruct((S, D), A_x.dtype),
        scratch_shapes=[
            pltpu.VMEM((S, D), A_x.dtype),
            pltpu.VMEM((D, 3 * D), A_wqkv.dtype),
            pltpu.VMEM((D, D), A_wo.dtype),
            pltpu.VMEM((D, F), B_w_gate.dtype),
            pltpu.VMEM((D, F), B_w_up.dtype),
            pltpu.VMEM((F, D), B_w_down.dtype),
            pltpu.VMEM((S, D), bf),
            pltpu.VMEM((D // 128, S, 128), bf),
            pltpu.VMEM((D, S), bf),
            pltpu.VMEM((D, TQ), bf),
            pltpu.VMEM((D, TQ), jnp.float32),
            pltpu.SemaphoreType.DMA((S // _RC + 7,)),
        ],
        compiler_params=pltpu.CompilerParams(
            dimension_semantics=("arbitrary",),
            vmem_limit_bytes=100 * 1024 * 1024),
    )(A_x.reshape(S, D), A_wqkv, A_wo, B_w_gate, B_w_up, B_w_down)
    return out.reshape(B, S, D)


@jax.jit
def pallas_parallel_sum__mha_block__swiglu_ffn__prompt_kernel(
    A_x, A_wqkv, A_wo, B_x, B_w_gate, B_w_up, B_w_down,
):
    return _call(A_x, A_wqkv, A_wo, B_w_gate, B_w_up, B_w_down)
```
